```python
import os as _os
_os.environ.setdefault("JAX_PLATFORMS", "cpu")
import jax
import jax.numpy as jnp

def _softmax(x, axis=-1):
    return jax.nn.softmax(x, axis=axis)
def _gelu(x):
    return jax.nn.gelu(x, approximate=True)
def _silu(x):
    return jax.nn.silu(x)
def _sigmoid(x):
    return jax.nn.sigmoid(x)
def _layernorm(x, axis=-1, eps=1e-5):
    m = jnp.mean(x, axis=axis, keepdims=True)
    v = jnp.var(x, axis=axis, keepdims=True)
    return (x - m) / jnp.sqrt(v + eps)
def _scatter_add(tgt, idx, src, axis=0):
    return tgt.at[idx].add(src)
def _segment_sum(src, seg, n):
    return jax.ops.segment_sum(src, seg, n)
class _Rng:
    def __init__(self, key):
        self._k = key
    def _next(self):
        self._k, sub = jax.random.split(self._k)
        return sub
    def normal(self, shape):
        return jax.random.normal(self._next(), shape, dtype=jnp.bfloat16)
    def randint(self, lo, hi, shape):
        return jax.random.randint(self._next(), shape, lo, hi, dtype=jnp.int32)
    def uniform(self, shape, lo=0.0, hi=1.0):
        return jax.random.uniform(self._next(), shape, jnp.bfloat16, lo, hi)
    def permutation(self, n):
        return jax.random.permutation(self._next(), n)


kernel_name = 'standalone__gqa_block_cached__sampling'

def setup_inputs():
    _rng = _Rng(jax.random.key(int.from_bytes(__import__("os").urandom(4), "little")))
    _w = (lambda a: (lambda t: t.astype(jnp.bfloat16) if jnp.issubdtype(t.dtype, jnp.floating) else t)(jnp.asarray(a)))
    B, Sq, D = 32, 16, 1024
    Hq, Hkv, Sk, Dh = 32, 4, 2048, 128
    assert Hq % Hkv == 0, (Hq, Hkv)
    return {
        "x": _w((lambda *s: _rng.normal(s) * 0.8)(B, Sq, D)),
        "k_cache": _w((lambda *s: _rng.normal(s) * 0.8)(B, Hkv, Sk, Dh)),
        "v_cache": _w((lambda *s: _rng.normal(s) * 0.05)(B, Hkv, Sk, Dh)),
        "wq": _w((lambda *s: _rng.normal(s) * 0.8)(D, Hq * Dh) * (D ** -0.5)),
        "wo": _w((lambda *s: _rng.normal(s) * 0.05)(Hq * Dh, D) * ((Hq * Dh) ** -0.5)),
    }

def reference(x, k_cache, v_cache, wq, wo):
    B, Sq, D = x.shape
    Hq, Dh = 32, 128
    Hkv = k_cache.shape[1]
    rep = Hq // Hkv
    q = (lambda x, *d: x.transpose(*d))((x @ wq).reshape(B, Sq, Hq, Dh), 0, 2, 1, 3)
    k = jnp.repeat(k_cache, rep, axis=1)
    v = jnp.repeat(v_cache, rep, axis=1)
    scores = jnp.einsum("bhqd,bhkd->bhqk", q, k) * (Dh ** -0.5)
    p = _softmax(scores, axis=-1)
    o = jnp.einsum("bhqk,bhkd->bhqd", p, v)
    return (lambda x, *d: x.transpose(*d))(o, 0, 2, 1, 3).reshape(B, Sq, Hq * Dh) @ wo
```

```python
import math
import functools
import jax
import jax.numpy as jnp
import jax.experimental.pallas as pl
import jax.experimental.pallas.tpu as pltpu

B, SQ, D = 32, 16, 1024
HQ, HKV, SK, DH = 32, 4, 2048, 128
REP = HQ // HKV
BB = 8
NBB = B // BB
ROWS = BB * SQ
NSS = HKV * NBB
NIT = NSS * BB
GW = REP * DH
QSCALE = (DH ** -0.5) * math.log2(math.e)
NT = (((1,), (1,)), ((), ()))


def make_kernel(NB=8, order="qk,qp,pv,op"):
    order = order.split(",")

    def kernel(x_hbm, k_hbm, v_hbm, wq_hbm, wo_hbm, out_hbm,
               xs, wqs, wos, kring, vring, qs, os_, acc, outs,
               kv_sem, w_sem, o_sem):
        def kv_copies(i, slot):
            g = i // (NBB * BB)
            b = i % (NBB * BB)
            return (pltpu.make_async_copy(k_hbm.at[b, g], kring.at[slot], kv_sem.at[0, slot]),
                    pltpu.make_async_copy(v_hbm.at[b, g], vring.at[slot], kv_sem.at[1, slot]))

        x_copy = pltpu.make_async_copy(x_hbm, xs, w_sem.at[0])

        def wq_copy(g):
            return pltpu.make_async_copy(wq_hbm.at[:, pl.ds(g * GW, GW)], wqs.at[g], w_sem.at[1 + g])

        def wo_copy(g):
            return pltpu.make_async_copy(wo_hbm.at[pl.ds(g * GW, GW), :], wos.at[g], w_sem.at[1 + HKV + g])

        def out_copy(bb):
            return pltpu.make_async_copy(outs.at[bb], out_hbm.at[pl.ds(bb * ROWS, ROWS), :], o_sem.at[bb])

        def qproj(ss, j):
            g = ss // NBB
            bb = ss % NBB
            c = pl.multiple_of(j * DH, DH)
            q = jnp.dot(xs[pl.ds(pl.multiple_of(bb * ROWS, ROWS), ROWS), :], wqs[g, :, pl.ds(c, DH)],
                        preferred_element_type=jnp.float32)
            q = (q * QSCALE).astype(jnp.bfloat16)
            qs[ss % 2, :, j] = q.reshape(BB, SQ, DH)

        def oproj(ss, j):
            g = ss // NBB
            bb = ss % NBB
            c = pl.multiple_of(j * DH, DH)
            upd = jnp.dot(os_[ss % 2], wos[g, :, pl.ds(c, DH)], preferred_element_type=jnp.float32)
            new = acc[bb, :, pl.ds(c, DH)] + upd
            acc[bb, :, pl.ds(c, DH)] = new
            outs[bb, :, pl.ds(c, DH)] = new.astype(jnp.bfloat16)

        x_copy.start()
        wq_copy(0).start()
        for i in range(NB):
            for c in kv_copies(i, i):
                c.start()
            if i == 1:
                wo_copy(0).start()
        acc[...] = jnp.zeros(acc.shape, jnp.float32)
        x_copy.wait()
        wq_copy(0).wait()

        def pro(j, _):
            qproj(0, j)
            return 0
        jax.lax.fori_loop(0, REP, pro, 0)

        def step(i, do_q, do_o):
            ss = i // BB
            j = i % BB
            slot = i % NB
            kc, vc = kv_copies(i, slot)
            st = {}

            def qk():
                kc.wait()
                q = qs[ss % 2, j].reshape(ROWS, DH)
                s = jax.lax.dot_general(q, kring[slot], NT, preferred_element_type=jnp.float32)
                st["s"] = s

            def pv():
                s = st["s"]
                m = jnp.max(s, axis=1, keepdims=True)
                p = jnp.exp2(s - m)
                l = jnp.sum(p, axis=1, keepdims=True)
                vc.wait()
                o = jnp.dot(p.astype(jnp.bfloat16), vring[slot], preferred_element_type=jnp.float32)
                o = (o * (1.0 / l)).astype(jnp.bfloat16)
                r = pl.multiple_of(j * SQ, SQ)
                for h in range(REP):
                    os_[ss % 2, pl.ds(r, SQ), h * DH:(h + 1) * DH] = o[h * SQ:(h + 1) * SQ, :]

            for name in order:
                if name == "qk":
                    qk()
                elif name == "pv":
                    pv()
                elif name == "qp" and do_q:
                    qproj(ss + 1, j)
                elif name == "op" and do_o:
                    oproj(ss - 1, j)

            @pl.when(i + NB < NIT)
            def _():
                for c in kv_copies(i + NB, slot):
                    c.start()

        sched = {8: [wq_copy(1)], 24: [wo_copy(1)], 40: [wq_copy(2)], 56: [wo_copy(2)],
                 72: [wq_copy(3)], 88: [wo_copy(3)]}

        def run(lo, hi, do_q, do_o):
            def body(i, _):
                step(i, do_q, do_o)
                for it, cps in sched.items():
                    if lo <= it < hi:
                        @pl.when(i == it)
                        def _():
                            for c in cps:
                                c.start()
                return 0
            jax.lax.fori_loop(lo, hi, body, 0)

        def waits(i, _unused=None):
            pass

        run(0, 8, True, False)
        wo_copy(0).wait()
        run(8, 24, True, True)
        wq_copy(1).wait()
        run(24, 40, True, True)
        wo_copy(1).wait()
        run(40, 56, True, True)
        wq_copy(2).wait()
        run(56, 72, True, True)
        wo_copy(2).wait()
        run(72, 88, True, True)
        wq_copy(3).wait()
        run(88, 104, True, True)
        wo_copy(3).wait()
        run(104, 120, True, True)
        run(120, 128, False, True)

        for bb in range(NBB - 1):
            out_copy(bb).start()

        def epi(j, _):
            oproj(NSS - 1, j)
            return 0
        jax.lax.fori_loop(0, REP, epi, 0)
        out_copy(NBB - 1).start()
        for bb in range(NBB):
            out_copy(bb).wait()

    return kernel


def build(NB=8, order="qk,qp,pv,op", vmem_mb=64, flags=None):
    kernel = make_kernel(NB, order)

    def fn(x, k_cache, v_cache, wq, wo):
        out = pl.pallas_call(
            kernel,
            in_specs=[pl.BlockSpec(memory_space=pl.ANY)] * 5,
            out_specs=pl.BlockSpec(memory_space=pl.ANY),
            out_shape=jax.ShapeDtypeStruct((B * SQ, D), jnp.bfloat16),
            scratch_shapes=[
                pltpu.VMEM((B * SQ, D), jnp.bfloat16),
                pltpu.VMEM((HKV, D, GW), jnp.bfloat16),
                pltpu.VMEM((HKV, GW, D), jnp.bfloat16),
                pltpu.VMEM((NB, SK, DH), jnp.bfloat16),
                pltpu.VMEM((NB, SK, DH), jnp.bfloat16),
                pltpu.VMEM((2, BB, REP, SQ, DH), jnp.bfloat16),
                pltpu.VMEM((2, ROWS, GW), jnp.bfloat16),
                pltpu.VMEM((NBB, ROWS, D), jnp.float32),
                pltpu.VMEM((NBB, ROWS, D), jnp.bfloat16),
                pltpu.SemaphoreType.DMA((2, NB)),
                pltpu.SemaphoreType.DMA((1 + 2 * HKV,)),
                pltpu.SemaphoreType.DMA((NBB,)),
            ],
            compiler_params=pltpu.CompilerParams(vmem_limit_bytes=vmem_mb << 20, flags=flags),
        )(x.reshape(B * SQ, D), k_cache, v_cache, wq, wo)
        return out.reshape(B, SQ, D)
    return fn


@jax.jit
def pallas_standalone__gqa_block_cached__sampling_kernel(
    x: jax.Array,
    k_cache: jax.Array,
    v_cache: jax.Array,
    wq: jax.Array,
    wo: jax.Array,
):
    return build(8, "qk,qp,op,pv")(x, k_cache, v_cache, wq, wo)
```

```python
import math
import contextlib
import jax
import jax.numpy as jnp
import jax.experimental.pallas as pl
import jax.experimental.pallas.tpu as pltpu

B, SQ, D = 32, 16, 1024
HQ, HKV, SK, DH = 32, 4, 2048, 128
REP = HQ // HKV
BB = 8
NBB = B // BB
ROWS = BB * SQ
NIT = HKV * B
GW = REP * DH
OB = 4
OROWS = OB * SQ
OCOLS = D // OB
QSCALE = (DH ** -0.5) * math.log2(math.e)
NT = (((1,), (1,)), ((), ()))
F32 = jnp.float32
BF16 = jnp.bfloat16
LAST = NIT - 1


def split_rows(total, n, align=16):
    base = (total // n) // align * align
    rem = (total - base * n) // align
    out, r0 = [], 0
    for r in range(n):
        s = base + (align if r < rem else 0)
        out.append((r0, s))
        r0 += s
    assert r0 == total
    return out


def make_kernel(S=5, NP=12, L=2, DK=2, DV=4, order="pv,qk,qp,op,sm", tailmap=(124, 124, 125, 125), lite=0, scopes=False,
                outp=1, outf=1, NS=None):
    WP = 16
    KVP = split_rows(SK, NP)
    WPB = GW // WP
    WPI = WPB // 16
    NPB = L + 1
    NS = L if NS is None else NS
    order = order.split(",")
    scope = (lambda n: jax.named_scope(n)) if scopes else (lambda n: contextlib.nullcontext())

    def kernel(x_hbm, k_hbm, v_hbm, wq_hbm, wo_hbm, out_hbm,
               xs, wqs, wos, kring, vring, qs, os_, pbuf, rbuf, acc, outs,
               kv_sem, w_sem, o_sem):
        def mo(v, n):
            return v if isinstance(v, int) else pl.multiple_of(v, n)

        def k_piece(i, r0, nr, prio=0):
            pltpu.make_async_copy(k_hbm.at[i % B, i // B, pl.ds(r0, nr)], kring.at[i % S, pl.ds(r0, nr)],
                                  kv_sem.at[0, i % S]).start(priority=prio)

        def v_piece(i, r0, nr, prio=1):
            pltpu.make_async_copy(v_hbm.at[i % B, i // B, pl.ds(r0, nr)], vring.at[i % S, pl.ds(r0, nr)],
                                  kv_sem.at[1, i % S]).start(priority=prio)

        def k_wait(i):
            pltpu.make_async_copy(kring.at[i % S], kring.at[i % S], kv_sem.at[0, i % S]).wait()

        def v_wait(i):
            pltpu.make_async_copy(vring.at[i % S], vring.at[i % S], kv_sem.at[1, i % S]).wait()

        def w_piece(blk, p, prio):
            r = mo(p * WP, WP)
            if blk < HKV:
                src, dst = wq_hbm.at[pl.ds(r, WP), pl.ds(blk * GW, GW)], wqs.at[blk, pl.ds(r, WP)]
            elif blk < 2 * HKV:
                g = blk - HKV
                src, dst = wo_hbm.at[pl.ds(g * GW + r, WP), :], wos.at[g, pl.ds(r, WP)]
            else:
                src, dst = x_hbm.at[pl.ds(r, WP), :], xs.at[pl.ds(r, WP)]
            pltpu.make_async_copy(src, dst, w_sem.at[blk]).start(priority=prio)

        def w_wait(blk):
            ref = wqs.at[blk] if blk < HKV else (wos.at[blk - HKV] if blk < 2 * HKV else xs)
            pltpu.make_async_copy(ref, ref, w_sem.at[blk]).wait()

        def issue(ki, vi, wblk=None, w0=None, nw=WPI, part=None, vsplit=False):
            every = NP // (nw // 2) if wblk is not None else None
            for r, (r0, nr) in enumerate(KVP):
                if part is not None and (r * 2) // NP != part:
                    continue
                if ki is not None:
                    k_piece(ki, r0, nr)
                if vi is not None:
                    v_piece(vi, r0, nr, (r % 2) if vsplit else 1)
                if wblk is not None and r % every == every // 2 and r // every < nw // 2:
                    w_piece(wblk, w0 + 2 * (r // every), 0)
                    w_piece(wblk, w0 + 2 * (r // every) + 1, 1)

        def out_piece(r0, nr, prio):
            pltpu.make_async_copy(outs.at[pl.ds(r0, nr)], out_hbm.at[pl.ds(r0, nr)], o_sem.at[0]).start(priority=prio)

        def qproj(ss, j):
            g = ss // NBB
            bb = ss % NBB
            q = jnp.dot(xs[pl.ds(mo(bb * ROWS, ROWS), ROWS), :], wqs[g, :, pl.ds(mo(j * DH, DH), DH)],
                        preferred_element_type=F32)
            q = (q * QSCALE).astype(BF16)
            qs[ss % 2, :, j] = q.reshape(BB, SQ, DH)

        def oproj(u, c0, nc):
            g = u // (B // OB)
            r = mo((u % (B // OB)) * OROWS, OROWS)
            c0 = mo(c0, nc)
            upd = jnp.dot(os_[u % 2], wos[g, :, pl.ds(c0, nc)], preferred_element_type=F32)
            new = acc[pl.ds(r, OROWS), pl.ds(c0, nc)] + upd
            acc[pl.ds(r, OROWS), pl.ds(c0, nc)] = new
            outs[pl.ds(r, OROWS), pl.ds(c0, nc)] = new.astype(BF16)

        def scores(i):
            q = qs[(i // BB) % 2, i % BB].reshape(ROWS, DH)
            return jax.lax.dot_general(q, kring[i % S], NT, preferred_element_type=F32)

        def softmax(i, s):
            m = jnp.max(s, axis=1, keepdims=True)
            p = jnp.exp2(s - m)
            l = jnp.sum(p, axis=1, keepdims=True)
            pbuf[i % NPB] = p.astype(BF16)
            rbuf[i % NPB] = jnp.broadcast_to(1.0 / l, (ROWS, DH))

        def pv(i):
            o = jnp.dot(pbuf[i % NPB], vring[i % S], preferred_element_type=F32)
            o = (o * rbuf[i % NPB]).astype(BF16)
            r = mo((i % OB) * SQ, SQ)
            for h in range(REP):
                os_[(i // OB) % 2, pl.ds(r, SQ), h * DH:(h + 1) * DH] = o[h * SQ:(h + 1) * SQ, :]

        if lite >= 1:
            _q, _o = qproj, oproj
            qproj = lambda ss, j: _q(ss, j) if isinstance(ss, int) else None
            oproj = lambda u, c0, nc: _o(u, c0, nc) if isinstance(u, int) else None
        if lite >= 3:
            scores = lambda i: None
            softmax = lambda i, s: None
            pv = lambda i: None
            qproj = lambda *a: None
            oproj = lambda *a: None

        for p in range(B * SQ // WP):
            w_piece(8, p, p % 2)
        for p in range(WPB):
            w_piece(0, p, p % 2)
        wo0 = list(range(WPB))

        def take_wo0(n, first_prio):
            for t in range(n):
                if wo0:
                    w_piece(HKV, wo0.pop(0), (first_prio + t) % 2)

        assert DK <= S and DV <= S
        nk0 = min(S, L + DK)
        kq = list(range(L + DK))
        vq = list(range(DV))
        for i in range(min(2, nk0)):
            ki = kq.pop(0)
            for (r0, nr) in KVP:
                k_piece(ki, r0, nr)
                take_wo0(1, 1)
        acc[...] = jnp.zeros(acc.shape, F32)
        w_wait(8)
        w_wait(0)

        def fill_one(nfree):
            ki = kq[0] if kq and kq[0] < nfree else None
            if ki is not None:
                kq.pop(0)
            vi = vq.pop(0) if vq else None
            if ki is not None or vi is not None:
                issue(ki, vi)

        for j in range(REP):
            qproj(0, j)
            if j % 2 == 1:
                fill_one(S)
            else:
                take_wo0(8, 0)
        take_wo0(len(wo0), 0)
        for i in range(L):
            k_wait(i)
            s_ = scores(i)
            qproj(1, i)
            softmax(i, s_)
            fill_one(S + i + 1)
        assert not kq
        while vq:
            fill_one(0)

        WSEQ = [1, HKV + 1, 2, HKV + 2, 3, HKV + 3]
        wwait = {4: HKV + 0, 24 - L: 1, 36: HKV + 1, 56 - L: 2, 68: HKV + 2, 88 - L: 3, 100: HKV + 3}

        def do_issue(i, lo, hi):
            w = lo // 16
            wblk = WSEQ[w] if w < len(WSEQ) else None
            w0 = (i - 16 * w) * WPI if wblk is not None else None
            first_split = NIT - NS
            if hi - 1 + DV < first_split and hi - 1 + DV <= LAST and hi - 1 + L + DK <= LAST:
                issue(i + L + DK, i + DV, wblk, w0)
                return
            assert wblk is None
            if hi - lo > 1 and NS == 0:
                kok, vok = hi - 1 + L + DK <= LAST, hi - 1 + DV <= LAST
                knone, vnone = lo + L + DK > LAST, lo + DV > LAST
                if knone and vnone:
                    return
                if kok or knone or vok or vnone:
                    pass
            for j in range(lo, hi):
                ki = j + L + DK if j + L + DK <= LAST else None
                vi = j + DV if j + DV <= LAST else None
                if ki is None and vi is None:
                    continue
                fn = lambda ki=ki, vi=vi: issue(ki, vi, vsplit=(vi is not None and vi >= first_split))
                if hi - lo == 1:
                    fn()
                else:
                    pl.when(i == j)(fn)

        def step(i, lo, hi, do_q, do_qk, opieces):
            for it, blk in wwait.items():
                if lo <= it < hi:
                    pl.when(i == it)(lambda: w_wait(blk))
            if do_qk:
                with scope("WAITK"):
                    k_wait(i + L)
            with scope("WAITV" if not isinstance(i, int) else f"WAITV{i}"):
                v_wait(i)
            st = {}
            for name in order:
                if name == "pv":
                    pv(i)
                elif name == "qk" and do_qk:
                    st["s"] = scores(i + L)
                elif name == "sm" and do_qk:
                    softmax(i + L, st["s"])
                elif name == "qp" and do_q:
                    qproj((i + L) // BB + 1, (i + L) % BB)
                elif name == "op":
                    if opieces == "std":
                        oproj(i // OB - 1, (i % OB) * OCOLS, OCOLS)
                    else:
                        for (u, c) in opieces:
                            oproj(u, c * OCOLS, OCOLS)
            do_issue(i, lo, hi)

        def loop(lo, hi, do_q, do_qk, opieces):
            if lo >= hi:
                return
            if hi - lo == 1:
                step(lo, lo, hi, do_q, do_qk, opieces)
                return
            def body(i, _):
                step(i, lo, hi, do_q, do_qk, opieces)
                return 0
            jax.lax.fori_loop(lo, hi, body, 0)

        E = NIT - BB - L
        U = NIT // OB - 2
        T0 = (U + 1) * OB
        loop(0, OB, True, True, [])
        loop(OB, 16, True, True, "std")
        for w in range(1, 6):
            loop(16 * w, 16 * w + 16, True, True, "std")
        loop(96, E, True, True, "std")
        R0 = max(E, min(T0, LAST - max(L + DK, DV + NS) + 1))
        loop(E, R0, False, True, "std")
        for i in range(R0, T0):
            loop(i, i + 1, False, i + L <= LAST, "std")
        nearly = B * SQ - OROWS
        for i in range(T0, NIT):
            pcs = [(U, c) for c in range(OB) if tailmap[c] == i]
            if i < LAST:
                loop(i, i + 1, False, i + L <= LAST, pcs)
            else:
                assert not pcs
                with scope(f"WAITV{i}"):
                    v_wait(i)
                for r, (r0, nr) in enumerate(split_rows(nearly, outp)):
                    out_piece(r0, nr, r % 2)
                pv(i)
        oproj(NIT // OB - 1, 0, D)
        for r, (r0, nr) in enumerate(split_rows(OROWS, outf)):
            out_piece(nearly + r0, nr, (r + 1) % 2)
        with scope("WAITO"):
            pltpu.make_async_copy(outs, outs, o_sem.at[0]).wait()

    return kernel


def build(vmem_mb=64, flags=None, nobc=True, **kw):
    kernel = make_kernel(**kw)
    S = kw.get("S", 5)
    L = kw.get("L", 2)

    def fn(x, k_cache, v_cache, wq, wo):
        out = pl.pallas_call(
            kernel,
            in_specs=[pl.BlockSpec(memory_space=pl.ANY)] * 5,
            out_specs=pl.BlockSpec(memory_space=pl.ANY),
            out_shape=jax.ShapeDtypeStruct((B * SQ, D), BF16),
            scratch_shapes=[
                pltpu.VMEM((B * SQ, D), BF16),
                pltpu.VMEM((HKV, D, GW), BF16),
                pltpu.VMEM((HKV, GW, D), BF16),
                pltpu.VMEM((S, SK, DH), BF16),
                pltpu.VMEM((S, SK, DH), BF16),
                pltpu.VMEM((2, BB, REP, SQ, DH), BF16),
                pltpu.VMEM((2, OROWS, GW), BF16),
                pltpu.VMEM((L + 1, ROWS, SK), BF16),
                pltpu.VMEM((L + 1, ROWS, DH), F32),
                pltpu.VMEM((B * SQ, D), F32),
                pltpu.VMEM((B * SQ, D), BF16),
                pltpu.SemaphoreType.DMA((2, S)),
                pltpu.SemaphoreType.DMA((2 * HKV + 1,)),
                pltpu.SemaphoreType.DMA((1,)),
            ],
            compiler_params=pltpu.CompilerParams(vmem_limit_bytes=vmem_mb << 20, flags=flags,
                                                 disable_bounds_checks=nobc),
        )(x.reshape(B * SQ, D), k_cache, v_cache, wq, wo)
        return out.reshape(B, SQ, D)
    return fn


@jax.jit
def pallas_standalone__gqa_block_cached__sampling_kernel(
    x: jax.Array,
    k_cache: jax.Array,
    v_cache: jax.Array,
    wq: jax.Array,
    wo: jax.Array,
):
    return build(NP=11, L=4, DK=3, DV=5, S=5, tailmap=(124, 125, 126, 126), outp=28, outf=4, NS=0)(
        x, k_cache, v_cache, wq, wo)
```

```python
import math

import jax
import jax.numpy as jnp
import jax.experimental.pallas as pl
import jax.experimental.pallas.tpu as pltpu

B, SQ, D = 32, 16, 1024
HQ, HKV, SK, DH = 32, 4, 2048, 128
REP = HQ // HKV
GW = REP * DH
NIT = HKV * B
LAST = NIT - 1

QB = 8
QROWS = QB * SQ
OB = 4
OROWS = OB * SQ
OCOLS = D // OB

SKEW = 5
SLOTS = 5
DK = 3
DV = 5
NPIECE = 11
WP = 16
WPB = GW // WP
WPI = 4

QSCALE = (DH ** -0.5) * math.log2(math.e)
NT = (((1,), (1,)), ((), ()))
F32 = jnp.float32
BF16 = jnp.bfloat16

WQ, WO, XB = 0, HKV, 2 * HKV
WSEQ = (WQ + 1, WO + 1, WQ + 2, WO + 2, WQ + 3, WO + 3)
WWAIT = {4: WO + 0, 24 - SKEW: WQ + 1, 36: WO + 1, 56 - SKEW: WQ + 2, 68: WO + 2, 88 - SKEW: WQ + 3, 100: WO + 3}

QEND = NIT - QB - SKEW
TAIL = 120
UL = NIT // OB - 1
TAIL_OPROJ = {
    120: ((UL - 2, 0), (UL - 2, 1)), 121: ((UL - 2, 2),), 122: ((UL - 2, 3),), 123: (),
    124: ((UL - 1, 0), (UL - 1, 1)), 125: ((UL - 1, 2),), 126: ((UL - 1, 3),),
}


def _split_rows(total, n, align=16):
    base = (total // n) // align * align
    rem = (total - base * n) // align
    out, r0 = [], 0
    for r in range(n):
        size = base + (align if r < rem else 0)
        out.append((r0, size))
        r0 += size
    assert r0 == total
    return out


KV_PIECES = _split_rows(SK, NPIECE)
W_AT = {(2 * t + 1) * NPIECE // WPI: t for t in range(WPI // 2)}


def _mo(v, n):
    return v if isinstance(v, int) else pl.multiple_of(v, n)


def _kernel(x_hbm, k_hbm, v_hbm, wq_hbm, wo_hbm, out_hbm,
            xs, wqs, wos, kring, vring, qs, os_, pbuf, rbuf, acc, outs,
            kv_sem, w_sem, o_sem):
    def k_piece(i, r0, nr):
        pltpu.make_async_copy(k_hbm.at[i % B, i // B, pl.ds(r0, nr)], kring.at[i % SLOTS, pl.ds(r0, nr)],
                              kv_sem.at[0, i % SLOTS]).start(priority=0)

    def v_piece(i, r0, nr):
        pltpu.make_async_copy(v_hbm.at[i % B, i // B, pl.ds(r0, nr)], vring.at[i % SLOTS, pl.ds(r0, nr)],
                              kv_sem.at[1, i % SLOTS]).start(priority=1)

    def k_wait(i):
        pltpu.make_async_copy(k_hbm.at[i % B, i // B], kring.at[i % SLOTS], kv_sem.at[0, i % SLOTS]).wait()

    def v_wait(i):
        pltpu.make_async_copy(v_hbm.at[i % B, i // B], vring.at[i % SLOTS], kv_sem.at[1, i % SLOTS]).wait()

    def w_refs(blk, rows):
        if blk < WO:
            return wq_hbm.at[rows, pl.ds(blk * GW, GW)], wqs.at[blk, rows]
        if blk < XB:
            g = blk - WO
            return wo_hbm.at[pl.ds(g * GW + rows.start, rows.size), :], wos.at[g, rows]
        return x_hbm.at[rows, :], xs.at[rows]

    def w_piece(blk, p, prio):
        src, dst = w_refs(blk, pl.ds(_mo(p * WP, WP), WP))
        pltpu.make_async_copy(src, dst, w_sem.at[blk]).start(priority=prio)

    def w_wait(blk):
        src, dst = w_refs(blk, pl.ds(0, B * SQ if blk == XB else GW))
        pltpu.make_async_copy(src, dst, w_sem.at[blk]).wait()

    def issue(ki, vi, wblk=None, w0=None):
        for r, (r0, nr) in enumerate(KV_PIECES):
            if ki is not None:
                k_piece(ki, r0, nr)
            if vi is not None:
                v_piece(vi, r0, nr)
            if wblk is not None and r in W_AT:
                w_piece(wblk, w0 + 2 * W_AT[r], 0)
                w_piece(wblk, w0 + 2 * W_AT[r] + 1, 1)

    def out_piece(p, prio):
        rows = pl.ds(p * WP, WP)
        pltpu.make_async_copy(outs.at[rows], out_hbm.at[rows], o_sem.at[0]).start(priority=prio)

    def qproj(ss, j):
        g, bb = ss // (B // QB), ss % (B // QB)
        q = jnp.dot(xs[pl.ds(_mo(bb * QROWS, QROWS), QROWS), :], wqs[g, :, pl.ds(_mo(j * DH, DH), DH)],
                    preferred_element_type=F32)
        qs[ss % 2, :, j] = (q * QSCALE).astype(BF16).reshape(QB, SQ, DH)

    def scores(i):
        q = qs[(i // QB) % 2, i % QB].reshape(REP * SQ, DH)
        return jax.lax.dot_general(q, kring[i % SLOTS], NT, preferred_element_type=F32)

    def softmax(i, s):
        m = jnp.max(s, axis=1, keepdims=True)
        p = jnp.exp2(s - m)
        l = jnp.sum(p, axis=1, keepdims=True)
        pbuf[i % (SKEW + 1)] = p.astype(BF16)
        rbuf[i % (SKEW + 1)] = jnp.broadcast_to(1.0 / l, (REP * SQ, DH))

    def pv(i):
        o = jnp.dot(pbuf[i % (SKEW + 1)], vring[i % SLOTS], preferred_element_type=F32)
        o = (o * rbuf[i % (SKEW + 1)]).astype(BF16)
        r = _mo((i % OB) * SQ, SQ)
        for h in range(REP):
            os_[(i // OB) % 2, pl.ds(r, SQ), h * DH:(h + 1) * DH] = o[h * SQ:(h + 1) * SQ, :]

    def oproj(u, c0, nc):
        g = u // (B // OB)
        r = _mo((u % (B // OB)) * OROWS, OROWS)
        c0 = _mo(c0, nc)
        new = acc[pl.ds(r, OROWS), pl.ds(c0, nc)] + jnp.dot(
            os_[u % 2], wos[g, :, pl.ds(c0, nc)], preferred_element_type=F32)
        acc[pl.ds(r, OROWS), pl.ds(c0, nc)] = new
        outs[pl.ds(r, OROWS), pl.ds(c0, nc)] = new.astype(BF16)

    for p in range(B * SQ // WP):
        w_piece(XB, p, p % 2)
    for p in range(WPB):
        w_piece(WQ, p, p % 2)
    wo0 = list(range(WPB))

    def take_wo0(n, prio):
        for t in range(min(n, len(wo0))):
            w_piece(WO, wo0.pop(0), (prio + t) % 2)

    kq = list(range(SKEW + DK))
    vq = list(range(DV))
    for _ in range(2):
        ki = kq.pop(0)
        for r0, nr in KV_PIECES:
            k_piece(ki, r0, nr)
            take_wo0(1, 1)
    acc[...] = jnp.zeros(acc.shape, F32)
    w_wait(XB)
    w_wait(WQ)

    def fill(nfree):
        ki = kq.pop(0) if kq and kq[0] < nfree else None
        vi = vq.pop(0) if vq else None
        if ki is not None or vi is not None:
            issue(ki, vi)

    for j in range(REP):
        qproj(0, j)
        if j % 2 == 1:
            fill(SLOTS)
        else:
            take_wo0(8, 0)
    take_wo0(WPB, 0)
    for i in range(SKEW):
        k_wait(i)
        s = scores(i)
        qproj(1, i)
        softmax(i, s)
        fill(SLOTS + i + 1)
    assert not kq and not vq and not wo0

    def block(i, lo, hi, do_q, opieces):
        for it, blk in WWAIT.items():
            if lo <= it < hi:
                pl.when(i == it)(lambda blk=blk: w_wait(blk))
        do_qk = hi - 1 + SKEW <= LAST
        assert do_qk or lo + SKEW > LAST
        if do_qk:
            k_wait(i + SKEW)
        v_wait(i)
        pv(i)
        if do_qk:
            s = scores(i + SKEW)
        if do_q:
            qproj((i + SKEW) // QB + 1, (i + SKEW) % QB)
        if opieces is None:
            oproj(i // OB - 1, (i % OB) * OCOLS, OCOLS)
        else:
            for u, c in opieces:
                oproj(u, c * OCOLS, OCOLS)
        if do_qk:
            softmax(i + SKEW, s)
        w = lo // 16
        assert (hi - 1) // 16 == w
        wblk = WSEQ[w] if w < len(WSEQ) else None
        ki = i + SKEW + DK if hi - 1 + SKEW + DK <= LAST else None
        vi = i + DV if hi - 1 + DV <= LAST else None
        assert ki is not None or lo + SKEW + DK > LAST
        assert vi is not None or lo + DV > LAST
        if ki is not None or vi is not None:
            issue(ki, vi, wblk, (i - 16 * w) * WPI if wblk is not None else None)

    def run(lo, hi, do_q, opieces):
        def body(i, carry):
            block(i, lo, hi, do_q, opieces)
            return carry
        jax.lax.fori_loop(lo, hi, body, 0)

    run(0, OB, True, ())
    run(OB, 16, True, None)
    for w in range(1, 6):
        run(16 * w, 16 * w + 16, True, None)
    run(96, 112, True, None)
    run(112, QEND, True, None)
    run(QEND, TAIL, False, None)
    for i in range(TAIL, LAST):
        block(i, i, i + 1, False, TAIL_OPROJ[i])

    v_wait(LAST)
    ndone = (B * SQ - OROWS) // WP
    for p in range(ndone):
        out_piece(p, p % 2)
    pv(LAST)
    oproj(UL, 0, D)
    for p in range(ndone, B * SQ // WP):
        out_piece(p, (p + 1) % 2)
    pltpu.make_async_copy(outs, out_hbm, o_sem.at[0]).wait()


@jax.jit
def pallas_standalone__gqa_block_cached__sampling_kernel(
    x: jax.Array,
    k_cache: jax.Array,
    v_cache: jax.Array,
    wq: jax.Array,
    wo: jax.Array,
):
    assert x.shape == (B, SQ, D) and k_cache.shape == v_cache.shape == (B, HKV, SK, DH)
    assert wq.shape == (D, HQ * DH) and wo.shape == (HQ * DH, D)
    out = pl.pallas_call(
        _kernel,
        in_specs=[pl.BlockSpec(memory_space=pl.ANY)] * 5,
        out_specs=pl.BlockSpec(memory_space=pl.ANY),
        out_shape=jax.ShapeDtypeStruct((B * SQ, D), x.dtype),
        scratch_shapes=[
            pltpu.VMEM((B * SQ, D), BF16),
            pltpu.VMEM((HKV, D, GW), BF16),
            pltpu.VMEM((HKV, GW, D), BF16),
            pltpu.VMEM((SLOTS, SK, DH), BF16),
            pltpu.VMEM((SLOTS, SK, DH), BF16),
            pltpu.VMEM((2, QB, REP, SQ, DH), BF16),
            pltpu.VMEM((2, OROWS, GW), BF16),
            pltpu.VMEM((SKEW + 1, REP * SQ, SK), BF16),
            pltpu.VMEM((SKEW + 1, REP * SQ, DH), F32),
            pltpu.VMEM((B * SQ, D), F32),
            pltpu.VMEM((B * SQ, D), BF16),
            pltpu.SemaphoreType.DMA((2, SLOTS)),
            pltpu.SemaphoreType.DMA((2 * HKV + 1,)),
            pltpu.SemaphoreType.DMA((1,)),
        ],
        compiler_params=pltpu.CompilerParams(
            vmem_limit_bytes=64 << 20,
            disable_bounds_checks=True,
            disable_semaphore_checks=True,
        ),
    )(x.reshape(B * SQ, D), k_cache, v_cache, wq, wo)
    return out.reshape(B, SQ, D)
```

```python
import math

import jax
import jax.numpy as jnp
import jax.experimental.pallas as pl
import jax.experimental.pallas.tpu as pltpu

B, SQ, D = 32, 16, 1024
HQ, HKV, SK, DH = 32, 4, 2048, 128
REP = HQ // HKV
GW = REP * DH
NIT = HKV * B
LAST = NIT - 1

QB = 8
QROWS = QB * SQ
OB = 4
OROWS = OB * SQ
OCOLS = D // OB

SKEW = 3
SLOTS = 5
DK = 3
DV = 5
WP = 16
WPB = GW // WP
WPI = 4

QSCALE = (DH ** -0.5) * math.log2(math.e)
NT = (((1,), (1,)), ((), ()))
F32 = jnp.float32
BF16 = jnp.bfloat16

WQ, WO, XB = 0, HKV, 2 * HKV
WSEQ = (WQ + 1, WO + 1, WQ + 2, WO + 2, WQ + 3, WO + 3)
WWAIT = {4: WO + 0, 24 - SKEW: WQ + 1, 36: WO + 1, 56 - SKEW: WQ + 2, 68: WO + 2, 88 - SKEW: WQ + 3, 100: WO + 3}

QEND = NIT - QB - SKEW
TAIL = 120
UL = NIT // OB - 1
TAIL_OPROJ = {
    120: ((UL - 2, 0), (UL - 2, 1)), 121: ((UL - 2, 2),), 122: ((UL - 2, 3),),
    123: ((UL - 1, 0), (UL - 1, 1), (UL - 1, 2)), 124: ((UL - 1, 3),), 125: (), 126: (),
}


KV_PIECES = ((1664, 256), (768, 128), (640, 128), (1408, 256), (128, 128), (256, 128), (1152, 128),
             (1280, 128), (384, 128), (512, 128), (896, 256), (0, 128), (1920, 128))
NPIECE = len(KV_PIECES)
assert sorted(r + t for r, n in KV_PIECES for t in range(0, n, 128)) == list(range(0, SK, 128))
W_AT = {(2 * t + 1) * NPIECE // WPI: t for t in range(WPI // 2)}


def _mo(v, n):
    return v if isinstance(v, int) else pl.multiple_of(v, n)


def _kernel(x_hbm, k_hbm, v_hbm, wq_hbm, wo_hbm, out_hbm,
            xs, wqs, wos, kring, vring, qs, os_, pbuf, rbuf, acc, outs,
            kv_sem, w_sem, o_sem):
    def k_piece(i, r0, nr):
        pltpu.make_async_copy(k_hbm.at[i % B, i // B, pl.ds(r0, nr)], kring.at[i % SLOTS, pl.ds(r0, nr)],
                              kv_sem.at[0, i % SLOTS]).start(priority=0)

    def v_piece(i, r0, nr):
        pltpu.make_async_copy(v_hbm.at[i % B, i // B, pl.ds(r0, nr)], vring.at[i % SLOTS, pl.ds(r0, nr)],
                              kv_sem.at[1, i % SLOTS]).start(priority=1)

    def k_wait(i):
        pltpu.make_async_copy(k_hbm.at[i % B, i // B], kring.at[i % SLOTS], kv_sem.at[0, i % SLOTS]).wait()

    def v_wait(i):
        pltpu.make_async_copy(v_hbm.at[i % B, i // B], vring.at[i % SLOTS], kv_sem.at[1, i % SLOTS]).wait()

    def w_refs(blk, rows):
        if blk < WO:
            return wq_hbm.at[rows, pl.ds(blk * GW, GW)], wqs.at[blk, rows]
        if blk < XB:
            g = blk - WO
            return wo_hbm.at[pl.ds(g * GW + rows.start, rows.size), :], wos.at[g, rows]
        return x_hbm.at[rows, :], xs.at[rows]

    def w_piece(blk, p, prio):
        src, dst = w_refs(blk, pl.ds(_mo(p * WP, WP), WP))
        pltpu.make_async_copy(src, dst, w_sem.at[blk]).start(priority=prio)

    def w_wait(blk):
        src, dst = w_refs(blk, pl.ds(0, B * SQ if blk == XB else GW))
        pltpu.make_async_copy(src, dst, w_sem.at[blk]).wait()

    def issue(ki, vi, wblk=None, w0=None):
        for r, (r0, nr) in enumerate(KV_PIECES):
            if vi is not None:
                v_piece(vi, r0, nr)
            if ki is not None:
                k_piece(ki, r0, nr)
            if wblk is not None and r in W_AT:
                w_piece(wblk, w0 + W_AT[r] + WPB // 2, 1)
                w_piece(wblk, w0 + W_AT[r], 0)

    def out_piece(p, prio):
        rows = pl.ds(p * WP, WP)
        pltpu.make_async_copy(outs.at[rows], out_hbm.at[rows], o_sem.at[0]).start(priority=prio)

    def qproj(ss, j):
        g, bb = ss // (B // QB), ss % (B // QB)
        q = jnp.dot(xs[pl.ds(_mo(bb * QROWS, QROWS), QROWS), :], wqs[g, :, pl.ds(_mo(j * DH, DH), DH)],
                    preferred_element_type=F32)
        qs[ss % 2, :, j] = (q * QSCALE).astype(BF16).reshape(QB, SQ, DH)

    def scores(i):
        q = qs[(i // QB) % 2, i % QB].reshape(REP * SQ, DH)
        return jax.lax.dot_general(q, kring[i % SLOTS], NT, preferred_element_type=F32)

    def softmax(i, s):
        m = jnp.max(s, axis=1, keepdims=True)
        p = jnp.exp2(s - m)
        l = jnp.sum(p, axis=1, keepdims=True)
        pbuf[i % (SKEW + 1)] = p.astype(BF16)
        rbuf[i % (SKEW + 1)] = jnp.broadcast_to(1.0 / l, (REP * SQ, DH))

    def pv(i):
        o = jnp.dot(pbuf[i % (SKEW + 1)], vring[i % SLOTS], preferred_element_type=F32)
        o = (o * rbuf[i % (SKEW + 1)]).astype(BF16)
        r = _mo((i % OB) * SQ, SQ)
        for h in range(REP):
            os_[(i // OB) % 2, pl.ds(r, SQ), h * DH:(h + 1) * DH] = o[h * SQ:(h + 1) * SQ, :]

    def oproj(u, c0, nc):
        g = u // (B // OB)
        r = _mo((u % (B // OB)) * OROWS, OROWS)
        c0 = _mo(c0, nc)
        new = acc[pl.ds(r, OROWS), pl.ds(c0, nc)] + jnp.dot(
            os_[u % 2], wos[g, :, pl.ds(c0, nc)], preferred_element_type=F32)
        acc[pl.ds(r, OROWS), pl.ds(c0, nc)] = new
        outs[pl.ds(r, OROWS), pl.ds(c0, nc)] = new.astype(BF16)

    nx = B * SQ // WP
    for p in range(nx):
        w_piece(WQ, p, 1)
        w_piece(XB, p, 0)
    for p in range(nx, (nx + WPB) // 2):
        w_piece(WQ, p + (WPB - nx) // 2, 1)
        w_piece(WQ, p, 0)
    wo0 = list(range(WPB))

    def take_wo0(n, prio):
        for t in range(min(n, len(wo0))):
            w_piece(WO, wo0.pop(0), (prio + t) % 2)

    kq = list(range(SKEW + DK))
    vq = list(range(DV))
    for _ in range(2):
        ki = kq.pop(0)
        for r0, nr in KV_PIECES:
            take_wo0(1, 1)
            k_piece(ki, r0, nr)
    acc[...] = jnp.zeros(acc.shape, F32)
    w_wait(XB)
    w_wait(WQ)

    def fill(nfree):
        ki = kq.pop(0) if kq and kq[0] < nfree else None
        vi = vq.pop(0) if vq else None
        if ki is not None or vi is not None:
            issue(ki, vi)

    for j in range(REP):
        qproj(0, j)
        if j % 2 == 1:
            fill(SLOTS)
        else:
            take_wo0(8, 0)
    take_wo0(WPB, 0)
    for i in range(SKEW):
        k_wait(i)
        s = scores(i)
        qproj(1, i)
        softmax(i, s)
        fill(SLOTS + i + 1)
    assert not kq and not vq and not wo0

    def block(i, lo, hi, do_q, opieces):
        for it, blk in WWAIT.items():
            if lo <= it < hi:
                pl.when(i == it)(lambda blk=blk: w_wait(blk))
        do_qk = hi - 1 + SKEW <= LAST
        assert do_qk or lo + SKEW > LAST
        if do_qk:
            k_wait(i + SKEW)
        v_wait(i)
        pv(i)
        if do_qk:
            s = scores(i + SKEW)
        if opieces is None:
            oproj(i // OB - 1, (i % OB) * OCOLS, OCOLS)
        else:
            for u, c in opieces:
                oproj(u, c * OCOLS, OCOLS)
        if do_q:
            qproj((i + SKEW) // QB + 1, (i + SKEW) % QB)
        if do_qk:
            softmax(i + SKEW, s)
        w = lo // 16
        assert (hi - 1) // 16 == w
        wblk = WSEQ[w] if w < len(WSEQ) else None
        ki = i + SKEW + DK if hi - 1 + SKEW + DK <= LAST else None
        vi = i + DV if hi - 1 + DV <= LAST else None
        assert ki is not None or lo + SKEW + DK > LAST
        assert vi is not None or lo + DV > LAST
        if ki is not None or vi is not None:
            issue(ki, vi, wblk, (i - 16 * w) * (WPI // 2) if wblk is not None else None)

    def run(lo, hi, do_q, opieces):
        def body(i, carry):
            block(i, lo, hi, do_q, opieces)
            return carry
        jax.lax.fori_loop(lo, hi, body, 0)

    run(0, OB, True, ())
    run(OB, 16, True, None)
    for w in range(1, 6):
        run(16 * w, 16 * w + 16, True, None)
    run(96, 112, True, None)
    run(112, QEND, True, None)
    run(QEND, TAIL, False, None)
    for i in range(TAIL, LAST):
        block(i, i, i + 1, False, TAIL_OPROJ[i])

    v_wait(LAST)
    ndone = (B * SQ - OROWS) // WP
    for p in range(ndone // 2):
        out_piece(p, 0)
        out_piece(p + ndone // 2, 1)
    pv(LAST)
    oproj(UL, 0, D)
    for p in range(ndone, B * SQ // WP):
        out_piece(p, (p + 1) % 2)
    pltpu.make_async_copy(outs, out_hbm, o_sem.at[0]).wait()


@jax.jit
def pallas_standalone__gqa_block_cached__sampling_kernel(
    x: jax.Array,
    k_cache: jax.Array,
    v_cache: jax.Array,
    wq: jax.Array,
    wo: jax.Array,
):
    assert x.shape == (B, SQ, D) and k_cache.shape == v_cache.shape == (B, HKV, SK, DH)
    assert wq.shape == (D, HQ * DH) and wo.shape == (HQ * DH, D)
    out = pl.pallas_call(
        _kernel,
        in_specs=[pl.BlockSpec(memory_space=pl.ANY)] * 5,
        out_specs=pl.BlockSpec(memory_space=pl.ANY),
        out_shape=jax.ShapeDtypeStruct((B * SQ, D), x.dtype),
        scratch_shapes=[
            pltpu.VMEM((B * SQ, D), BF16),
            pltpu.VMEM((HKV, D, GW), BF16),
            pltpu.VMEM((HKV, GW, D), BF16),
            pltpu.VMEM((SLOTS, SK, DH), BF16),
            pltpu.VMEM((SLOTS, SK, DH), BF16),
            pltpu.VMEM((2, QB, REP, SQ, DH), BF16),
            pltpu.VMEM((2, OROWS, GW), BF16),
            pltpu.VMEM((SKEW + 1, REP * SQ, SK), BF16),
            pltpu.VMEM((SKEW + 1, REP * SQ, DH), F32),
            pltpu.VMEM((B * SQ, D), F32),
            pltpu.VMEM((B * SQ, D), BF16),
            pltpu.SemaphoreType.DMA((2, SLOTS)),
            pltpu.SemaphoreType.DMA((2 * HKV + 1,)),
            pltpu.SemaphoreType.DMA((1,)),
        ],
        compiler_params=pltpu.CompilerParams(
            vmem_limit_bytes=64 << 20,
            disable_bounds_checks=True,
            disable_semaphore_checks=True,
        ),
    )(x.reshape(B * SQ, D), k_cache, v_cache, wq, wo)
    return out.reshape(B, SQ, D)
```
